```python
import os as _os
_os.environ.setdefault("JAX_PLATFORMS", "cpu")
import jax
import jax.numpy as jnp

def _softmax(x, axis=-1):
    return jax.nn.softmax(x, axis=axis)
def _gelu(x):
    return jax.nn.gelu(x, approximate=True)
def _silu(x):
    return jax.nn.silu(x)
def _sigmoid(x):
    return jax.nn.sigmoid(x)
def _layernorm(x, axis=-1, eps=1e-5):
    m = jnp.mean(x, axis=axis, keepdims=True)
    v = jnp.var(x, axis=axis, keepdims=True)
    return (x - m) / jnp.sqrt(v + eps)
def _scatter_add(tgt, idx, src, axis=0):
    return tgt.at[idx].add(src)
def _segment_sum(src, seg, n):
    return jax.ops.segment_sum(src, seg, n)
class _Rng:
    def __init__(self, key):
        self._k = key
    def _next(self):
        self._k, sub = jax.random.split(self._k)
        return sub
    def normal(self, shape):
        return jax.random.normal(self._next(), shape, dtype=jnp.bfloat16)
    def randint(self, lo, hi, shape):
        return jax.random.randint(self._next(), shape, lo, hi, dtype=jnp.int32)
    def uniform(self, shape, lo=0.0, hi=1.0):
        return jax.random.uniform(self._next(), shape, jnp.bfloat16, lo, hi)
    def permutation(self, n):
        return jax.random.permutation(self._next(), n)


kernel_name = 'interleave_layers__sliding_local_dilated__linear_kernel_hedgehog__prompt'

def setup_inputs():
    _rng = _Rng(jax.random.key(int.from_bytes(__import__("os").urandom(4), "little")))
    _w = (lambda a: (lambda t: t.astype(jnp.bfloat16) if jnp.issubdtype(t.dtype, jnp.floating) else t)(jnp.asarray(a)))
    def _A_setup():
        B, S, D = 1, 2048, 640
        return {
            "x": _w((lambda *s: _rng.normal(s) * 0.05)(B, S, D)),
            "wqkv": _w((lambda *s: _rng.normal(s) * 0.05)(D, 3 * D)),
            "wo": _w((lambda *s: _rng.normal(s) * 0.05)(D, D)),
        }
    _A_in = _A_setup()

    def _B_setup():
        B, S, D, H = 1, 2048, 640, 32
        Dh = D // H
        return {
            "x": _w((lambda *s: _rng.normal(s) * 0.05)(B, S, D)),
            "wqkv": _w((lambda *s: _rng.normal(s) * 0.4)(D, 3 * D)),
            "w_phi": _w((lambda *s: _rng.normal(s) * 0.4)(H, Dh, Dh) * (Dh ** -0.5)),
            "wo": _w((lambda *s: _rng.normal(s) * 0.1)(D, D)),
        }
    _B_in = _B_setup()

    return {
        "A_x": _A_in["x"],
        "A_wqkv": _A_in["wqkv"],
        "A_wo": _A_in["wo"],
        "B_x": _B_in["x"],
        "B_wqkv": _B_in["wqkv"],
        "B_w_phi": _B_in["w_phi"],
        "B_wo": _B_in["wo"],
    }

def reference(A_x, A_wqkv, A_wo, B_x, B_wqkv, B_w_phi, B_wo):
    def _A_ref(x, wqkv, wo):
        B, S, D = x.shape
        H = 32; Dh = D // H
        W, dil = 8, 2
        qkv = (lambda x, *d: x.transpose(*d))((x @ wqkv).reshape(B, S, 3, H, Dh), 2, 0, 3, 1, 4)
        q, k, v = qkv[0], qkv[1], qkv[2]
        scale = Dh ** -0.5
        pos = jnp.arange(S)
        off = jnp.arange(W) * dil
        idx = pos[:, None] - off[None, :]
        mask = idx >= 0
        idx_c = jnp.where(mask, idx, 0).reshape(-1)
        kg = k[:, :, idx_c, :].reshape(B, H, S, W, Dh)
        vg = v[:, :, idx_c, :].reshape(B, H, S, W, Dh)
        logits = jnp.einsum("bhsd,bhswd->bhsw", q, kg) * scale
        logits = jnp.where(mask[None, None, :, :], logits, -1e9)
        attn = _softmax(logits, axis=-1)
        o = jnp.einsum("bhsw,bhswd->bhsd", attn, vg)
        return (lambda x, *d: x.transpose(*d))(o, 0, 2, 1, 3).reshape(B, S, D) @ wo

    def _B_ref(x, wqkv, w_phi, wo):
        B, S, D = x.shape
        H = 32; Dh = D // H
        qkv = (lambda x, *d: x.transpose(*d))((x @ wqkv).reshape(B, S, 3, H, Dh), 2, 0, 3, 1, 4)
        q, k, v = qkv[0], qkv[1], qkv[2]
        pq = jnp.einsum("bhsd,hdf->bhsf", q, w_phi)
        pk = jnp.einsum("bhsd,hdf->bhsf", k, w_phi)
        phi_q = jnp.concatenate([_softmax(pq, axis=-1), _softmax(-pq, axis=-1)], axis=-1)
        phi_k = jnp.concatenate([_softmax(pk, axis=-1), _softmax(-pk, axis=-1)], axis=-1)
        kv = jnp.einsum("bhsf,bhsd->bhfd", phi_k, v)
        z  = jnp.einsum("bhsf->bhf", phi_k)
        num = jnp.einsum("bhqf,bhfd->bhqd", phi_q, kv)
        den = jnp.einsum("bhqf,bhf->bhq", phi_q, z)[..., None] + 1e-6
        o = num / den
        return (lambda x, *d: x.transpose(*d))(o, 0, 2, 1, 3).reshape(B, S, D) @ wo

    x = A_x
    x = x + _A_ref(_layernorm(x, axis=-1), A_wqkv, A_wo)
    x = x + _B_ref(_layernorm(x, axis=-1), B_wqkv, B_w_phi, B_wo)
    x = x + _A_ref(_layernorm(x, axis=-1), A_wqkv, A_wo)
    x = x + _B_ref(_layernorm(x, axis=-1), B_wqkv, B_w_phi, B_wo)
    return x
```

```python
import functools
import math
import jax
import jax.numpy as jnp
from jax import lax
import jax.experimental.pallas as pl
import jax.experimental.pallas.tpu as pltpu

S, D, H, DH = 2048, 640, 32, 20
T = 16
L = 128
G = 4
GR = 160
LOG2E = math.log2(math.e)
f32, bf16, u32 = jnp.float32, jnp.bfloat16, jnp.uint32
NT = (((1,), (1,)), ((), ()))


def _pk(x):
    return pltpu.bitcast(x.astype(bf16), u32)


def _up(x):
    return pltpu.bitcast(x, bf16)


def _ln(x):
    m = jnp.sum(x, axis=0, keepdims=True) * (1.0 / D)
    c = x - m
    v = jnp.sum(c * c, axis=0, keepdims=True) * (1.0 / D)
    return _pk(c * lax.rsqrt(v + 1e-5))


def _prep_plain(w_ref, col0, tmp, dst, row0, scale=None):
    for it in range(5):
        for ct in range(5):
            blk = w_ref[it * L:(it + 1) * L, col0 + ct * L:col0 + (ct + 1) * L].astype(f32)
            tmp[it, ct * L:(ct + 1) * L, :] = blk.T
        for g in range(G):
            for d in range(0, DH, 2):
                a = tmp[it, pl.ds(g * GR + d, 8, stride=DH), :]
                b = tmp[it, pl.ds(g * GR + d + 1, 8, stride=DH), :]
                r = jnp.concatenate([a, b], axis=0)
                if scale is not None:
                    r = r * scale
                dst[pl.ds((row0 + g * GR + d * 8) // 2, 8), it * L:(it + 1) * L] = _pk(r)
        yield


def _prep_wo(w_ref, tmp, tmp2, dst):
    for ot in range(5):
        tmp[ot] = w_ref[:, ot * L:(ot + 1) * L].astype(f32)
        for g in range(G):
            for d in range(DH):
                tmp2[ot, pl.ds(g * GR + d * 8, 8), :] = tmp[ot, pl.ds(g * GR + d, 8, stride=DH), :]
        for rt in range(5):
            blk = tmp2[ot, rt * L:(rt + 1) * L, :]
            dst[ot * 64:(ot + 1) * 64, rt * L:(rt + 1) * L] = _pk(blk.T)
        yield


def _prep_phi(wphi_ref, tmp, tmp2, pm):
    a = tmp.at[0]
    a[0:DH * 24, :] = jnp.zeros((DH * 24, L), f32)
    for d in range(DH):
        a[d * 24:d * 24 + DH, 0:H] = wphi_ref[d].astype(f32) * LOG2E
    lane = lax.broadcasted_iota(jnp.int32, (L, L), 1)
    row = lax.broadcasted_iota(jnp.int32, (L, L), 0)
    for f4 in range(5):
        m = None
        for fi in range(4):
            t = a[pl.ds(4 * f4 + fi, DH, stride=24), :]
            t = pltpu.roll(t, 32 * fi, 1) if fi else t
            m = t if m is None else m + t
        for h2 in range(16):
            tmp2[f4, pl.ds(2 * DH * h2, DH), :] = m
            tmp2[f4, pl.ds(2 * DH * h2 + DH, DH), :] = m
    yield
    lo = (lane & 31) * DH
    for ct in range(5):
        c = row + ct * L
        msk = (c >= lo) & (c < lo + DH)
        for f4 in range(5):
            y = jnp.where(msk, tmp2[f4, ct * L:(ct + 1) * L, :], 0.0).T
            for g in range(G):
                if g <= ct <= g + 1:
                    for fi in (0, 2):
                        r = jnp.concatenate([y[32 * fi + 8 * g:32 * fi + 8 * g + 8],
                                             y[32 * fi + 32 + 8 * g:32 * fi + 40 + 8 * g]], axis=0)
                        pm[g, pl.ds((4 * f4 + fi) * 8, 16), (ct - g) * L:(ct - g + 1) * L] = r.astype(bf16)
        yield


def _phi(p_ref, dst, groups=range(G)):
    for g in groups:
        p = p_ref[pl.ds(g * GR, GR), :].reshape(DH, 8, L)
        mx = jnp.max(p, axis=0, keepdims=True)
        mn = jnp.min(p, axis=0, keepdims=True)
        ep = jnp.exp2(p - mx)
        rp = 1.0 / jnp.sum(ep, axis=0, keepdims=True)
        dst[g, 0:80, :] = _pk((ep * rp).reshape(GR, L))
        en = jnp.exp2(mn - p)
        rn = 1.0 / jnp.sum(en, axis=0, keepdims=True)
        dst[g, 80:GR, :] = _pk((en * rn).reshape(GR, L))


def _dot(a, b):
    return jnp.dot(a, b, preferred_element_type=f32)


def _pipeline(stages, lo_extra, hi_extra):
    mx = max(o for _, o in stages)
    mn = min(o for _, o in stages)

    def body(a, c):
        for fn, o in stages:
            fn(a + o)
        return c
    for a in range(-mx, -mn):
        for fn, o in stages:
            if 0 <= a + o < T:
                fn(a + o)
    lax.fori_loop(-mn, T - mx, body, 0)
    for a in range(T - mx, T - mn):
        for fn, o in stages:
            if 0 <= a + o < T:
                fn(a + o)


def _kernel(x_hbm, aw_hbm, awo_hbm, bw_hbm, wphi_ref, bwo_hbm, o_hbm,
            xio, aw, awo, bw, bwo, WA, WAO, WB, WBO, PM, tmp, tmp2,
            X, XN, XN2, K, V, Q, PK, PV, Y, O, PHI, VG, KV, KVB, sems):
    cp_x = [pltpu.make_async_copy(x_hbm.at[:, ct * L:(ct + 1) * L], xio.at[ct], sems.at[5 + ct]) for ct in range(5)]
    cp_kv = pltpu.make_async_copy(aw_hbm.at[:, D:], aw.at[:, D:], sems.at[0])
    cp_aw = pltpu.make_async_copy(aw_hbm.at[:, :D], aw.at[:, :D], sems.at[1])
    cp_awo = pltpu.make_async_copy(awo_hbm, awo, sems.at[2])
    cp_bw = pltpu.make_async_copy(bw_hbm, bw, sems.at[3])
    cp_bwo = pltpu.make_async_copy(bwo_hbm, bwo, sems.at[4])
    cp_kv.start()
    for c in cp_x:
        c.start()
    cp_aw.start()
    cp_awo.start()
    cp_bw.start()
    cp_bwo.start()

    sub8 = lax.broadcasted_iota(jnp.int32, (8, L), 0)
    ones_pad = jnp.where(sub8 < 4, jnp.uint32(0x3F803F80), jnp.uint32(0))
    for g in range(G):
        PHI[g, GR:192, :] = jnp.zeros((32, L), u32)
        VG[g, 80:88, :] = ones_pad

    x32 = xio.bitcast(u32)

    def ldx(jj):
        for ct in range(5):
            u = x32[ct, pl.ds(jj, L, stride=8), :].T
            X[2 * jj, ct * L:(ct + 1) * L, :] = pltpu.bitcast(u << 16, f32)
            X[2 * jj + 1, ct * L:(ct + 1) * L, :] = pltpu.bitcast(u & jnp.uint32(0xFFFF0000), f32)

    def rest():
        yield from _prep_plain(aw, 0, tmp, WA, 0, scale=DH ** -0.5 * LOG2E)
        yield from _prep_wo(awo, tmp, tmp2, WAO)
        yield from _prep_phi(wphi_ref, tmp, tmp2, PM)
        for part in range(2):
            for g in range(G):
                r = lax.dot_general(PM[g], bw[:, part * D + g * L:part * D + g * L + 256], NT,
                                    preferred_element_type=f32)
                WB[pl.ds((part * D + g * GR) // 2, 80), :] = _pk(r)
        yield from _prep_plain(bw, 2 * D, tmp, WB, 2 * D)
        yield from _prep_wo(bwo, tmp, tmp2, WBO)

    def ln0(j):
        XN[j] = _ln(X[j])

    def kproj(j):
        k = _dot(_up(WA[320:640, :]), _up(XN[j]))
        K[j + T] = k
        K[j] = pltpu.roll(k, 1, 1)

    def vproj(j):
        v = _dot(_up(WA[640:960, :]), _up(XN[j]))
        V[j + T] = v
        V[j] = pltpu.roll(v, 1, 1)

    lane0 = lax.broadcasted_iota(jnp.int32, (8, L), 1) == 0

    def qproj(W):
        def fn(j):
            Q[j & 1] = _dot(_up(W[0:320, :]), _up(XN[j]))
        return fn

    def attn(groups):
        def fn(j):
            for g in groups:
                rows = pl.ds(g * GR, GR)
                q = Q[j & 1, rows, :].reshape(DH, 8, L)
                ls = []
                for w in range(8):
                    k = K[j + T - 2 * w, rows, :].reshape(DH, 8, L)
                    l = jnp.sum(q * k, axis=0)
                    if w > 0:
                        l = jnp.where(lane0 & (j < 2 * w), -1e9 * LOG2E, l)
                    ls.append(l)
                m = functools.reduce(jnp.maximum, ls)
                es = [jnp.exp2(l - m) for l in ls]
                r = 1.0 / functools.reduce(jnp.add, es)
                o = None
                for w in range(8):
                    v = V[j + T - 2 * w, rows, :].reshape(DH, 8, L)
                    t = (es[w] * r)[None] * v
                    o = t if o is None else o + t
                O[j & 1, pl.ds(g * 80, 80), :] = _pk(o.reshape(GR, L))
        return fn

    def oproj(W):
        def fn(j):
            X[j] = X[j] + _dot(_up(W[...]), _up(O[j & 1]))
        return fn

    def ln2(j):
        XN2[...] = _ln(X[j])
        XN[j] = XN2[...]

    def bk(h):
        def fn(j):
            PK[h * 320:(h + 1) * 320] = _dot(_up(WB[320 + 160 * h:480 + 160 * h, :]), _up(XN2[...]))
        return fn

    def bv(h):
        def fn(j):
            v = _pk(_dot(_up(WB[640 + 160 * h:800 + 160 * h, :]), _up(XN2[...])))
            for g in range(2):
                VG[2 * h + g, 0:80, :] = v[g * 80:(g + 1) * 80]
        return fn

    def phi2(h):
        return lambda j: _phi(PK, PHI, (2 * h, 2 * h + 1))

    def kvacc(j):
        for g in range(G):
            KV[g] += lax.dot_general(_up(VG[g]), _up(PHI[g]), NT, preferred_element_type=f32)

    def b_finish():
        r = lax.broadcasted_iota(jnp.int32, (176, 384), 0)
        c = lax.broadcasted_iota(jnp.int32, (176, 384), 1)
        m = (r & 7) == (c & 7)
        for g in range(G):
            KVB[g] = _pk(jnp.where(m, KV[g], 0.0))

    def phiq(j):
        _phi(Q.at[j & 1], PHI)

    def numm(j):
        for g in range(G):
            num = _dot(_up(KVB[g]), _up(PHI[g]))
            rd = 1.0 / (num[GR:GR + 8] + 1e-6)
            O[j & 1, pl.ds(g * 80, 80), :] = _pk((num[0:GR].reshape(DH, 8, L) * rd[None]).reshape(GR, L))

    cp_kv.wait()
    for part in (1, 2):
        for _ in _prep_plain(aw, part * D, tmp, WA, part * D):
            pass
    for c in cp_x:
        c.wait()
    ldx(0)
    ln0(0)
    gen = rest()
    for j in range(T):
        if j == 2:
            cp_aw.wait()
            cp_awo.wait()
        if j == 6:
            cp_bw.wait()
            cp_bwo.wait()
        kproj(j)
        if j % 2 == 0 and j + 2 < T:
            ldx(j // 2 + 1)
        if j >= 2:
            next(gen, None)
        vproj(j)
        if j + 1 < T:
            ln0(j + 1)
        if j >= 2:
            next(gen, None)
    for _ in gen:
        pass
    for rep in range(2):
        KV[...] = jnp.zeros(KV.shape, f32)
        _pipeline([(oproj(WAO), 0), (attn((0, 1)), 1), (qproj(WA), 2), (ln2, 0), (bk(0), 0), (attn((2,)), 1), (bk(1), 0), (phi2(0), 0),
                   (bv(0), 0), (attn((3,)), 1), (bv(1), 0), (phi2(1), 0), (kvacc, 0)], 0, 0)
        b_finish()
        if rep == 0:
            _pipeline([(oproj(WBO), 0), (phiq, 1), (qproj(WB), 2), (ln0, 0), (numm, 1), (kproj, 0), (vproj, 0)], 0, 0)
        else:
            _pipeline([(oproj(WBO), 0), (phiq, 1), (qproj(WB), 2), (numm, 1)], 0, 0)

    for jj in range(T // 2):
        for ct in range(5):
            lo = pltpu.bitcast(X[2 * jj, ct * L:(ct + 1) * L, :].astype(bf16).astype(f32), u32)
            hi = pltpu.bitcast(X[2 * jj + 1, ct * L:(ct + 1) * L, :].astype(bf16).astype(f32), u32)
            x32[ct, pl.ds(jj, L, stride=8), :] = (hi | (lo >> 16)).T
    cp_o = [pltpu.make_async_copy(xio.at[ct], o_hbm.at[:, ct * L:(ct + 1) * L], sems.at[5 + ct]) for ct in range(5)]
    for c in cp_o:
        c.start()
    for c in cp_o:
        c.wait()


@jax.jit
def pallas_interleave_layers__sliding_local_dilated__linear_kernel_hedgehog__prompt_kernel(
        A_x, A_wqkv, A_wo, B_x, B_wqkv, B_w_phi, B_wo):
    anyspec = pl.BlockSpec(memory_space=pl.ANY)
    V = pltpu.VMEM
    out = pl.pallas_call(
        _kernel,
        out_shape=jax.ShapeDtypeStruct((S, D), bf16),
        in_specs=[anyspec, anyspec, anyspec, anyspec,
                  pl.BlockSpec(memory_space=pltpu.VMEM), anyspec],
        out_specs=anyspec,
        scratch_shapes=[
            V((5, S, L), bf16), V((D, 3 * D), bf16), V((D, D), bf16), V((D, 3 * D), bf16), V((D, D), bf16),
            V((960, D), u32), V((320, D), u32), V((960, D), u32), V((320, D), u32),
            V((G, GR, 256), bf16), V((5, D, L), f32), V((5, D, L), f32),
            V((T, D, L), f32), V((T, 320, L), u32), V((320, L), u32), V((2 * T, D, L), f32), V((2 * T, D, L), f32),
            V((2, D, L), f32), V((D, L), f32), V((D, L), f32), V((D, L), f32),
            V((2, 320, L), u32), V((G, 192, L), u32), V((G, 88, L), u32),
            V((G, 176, 384), f32), V((G, 88, 384), u32),
            pltpu.SemaphoreType.DMA((10,)),
        ],
        compiler_params=pltpu.CompilerParams(vmem_limit_bytes=100 * 2 ** 20),
    )(A_x.reshape(S, D), A_wqkv, A_wo, B_wqkv, B_w_phi.transpose(1, 2, 0), B_wo)
    return out.reshape(1, S, D)
```
